```python
import os as _os
_os.environ.setdefault('JAX_PLATFORMS', 'cpu')
import jax
import jax.numpy as jnp

def _softmax(x, axis=-1):
    return jax.nn.softmax(x, axis=axis)

def _gelu(x):
    return jax.nn.gelu(x, approximate=True)

def _silu(x):
    return jax.nn.silu(x)

def _sigmoid(x):
    return jax.nn.sigmoid(x)

def _layernorm(x, axis=-1, eps=1e-05):
    m = jnp.mean(x, axis=axis, keepdims=True)
    v = jnp.var(x, axis=axis, keepdims=True)
    return (x - m) / jnp.sqrt(v + eps)

def _scatter_add(tgt, idx, src, axis=0):
    return tgt.at[idx].add(src)

def _segment_sum(src, seg, n):
    return jax.ops.segment_sum(src, seg, n)

class _Rng:

    def __init__(self, key):
        self._k = key

    def _next(self):
        self._k, sub = jax.random.split(self._k)
        return sub

    def normal(self, shape):
        return jax.random.normal(self._next(), shape, dtype=jnp.bfloat16)

    def randint(self, lo, hi, shape):
        return jax.random.randint(self._next(), shape, lo, hi, dtype=jnp.int32)

    def uniform(self, shape, lo=0.0, hi=1.0):
        return jax.random.uniform(self._next(), shape, jnp.bfloat16, lo, hi)

    def permutation(self, n):
        return jax.random.permutation(self._next(), n)
kernel_name = 'gated_mix__memory_aug_recurrent_mem_tr__glu_gated_geglu__prompt'

def setup_inputs():
    _rng = _Rng(jax.random.key(int.from_bytes(__import__("os").urandom(4), "little")))
    _w = lambda a: (lambda t: t.astype(jnp.bfloat16) if jnp.issubdtype(t.dtype, jnp.floating) else t)(jnp.asarray(a))

    def _A_setup():
        B, S, Dm = (1, 2048, 640)
        H, Dh = (32, 128)
        M, seg = (8, 32)
        seg = min(seg, S)
        S = S // seg * seg
        return {'x': _w((lambda *s: _rng.normal(s) * 0.05)(B, S, Dm)), 'mem0': _w((lambda *s: _rng.normal(s) * 0.4)(B, M, Dm)), 'Wq': _w((lambda *s: _rng.normal(s) * 3.2)(Dm, H, Dh) * Dm ** (-0.5)), 'Wk': _w((lambda *s: _rng.normal(s) * 3.2)(Dm, H, Dh) * Dm ** (-0.5)), 'Wv': _w((lambda *s: _rng.normal(s) * 0.4)(Dm, H, Dh) * Dm ** (-0.5)), 'Wo': _w((lambda *s: _rng.normal(s) * 0.4)(H, Dh, Dm) * (H * Dh) ** (-0.5)), 'seg_len': seg}
    _A_in = _A_setup()

    def _B_setup():
        B, S, Dm, Df = (1, 2048, 640, 1728)
        return {'x': _w((lambda *s: _rng.normal(s) * 0.05)(B, S, Dm)), 'w_gate': _w((lambda *s: _rng.normal(s) * 1.6)(Dm, Df) * Dm ** (-0.5)), 'w_up': _w((lambda *s: _rng.normal(s) * 1.6)(Dm, Df) * Dm ** (-0.5)), 'w_down': _w((lambda *s: _rng.normal(s) * 1.6)(Df, Dm) * Df ** (-0.5))}
    _B_in = _B_setup()
    return {'A_x': _A_in['x'], 'A_mem0': _A_in['mem0'], 'A_Wq': _A_in['Wq'], 'A_Wk': _A_in['Wk'], 'A_Wv': _A_in['Wv'], 'A_Wo': _A_in['Wo'], 'A_seg_len': _A_in['seg_len'], 'B_x': _B_in['x'], 'B_w_gate': _B_in['w_gate'], 'B_w_up': _B_in['w_up'], 'B_w_down': _B_in['w_down'], 'gate_w': _w((lambda *s: _rng.normal(s) * 0.05)(640) * 16.0)}

def reference(A_x, A_mem0, A_Wq, A_Wk, A_Wv, A_Wo, A_seg_len, B_x, B_w_gate, B_w_up, B_w_down, gate_w):

    def _A_ref(x, mem0, Wq, Wk, Wv, Wo, seg_len):
        B, S, Dm = x.shape
        H, Dh = (Wq.shape[1], Wq.shape[2])
        M = mem0.shape[1]
        scale = Dh ** (-0.5)
        n_seg = S // seg_len
        L = M + seg_len
        idx = jnp.arange(L)
        mask = (idx[:, None] < M) | (idx[:, None] >= idx[None, :])
        mem = mem0
        outs = []
        for s in range(n_seg):
            xs = x[:, s * seg_len:(s + 1) * seg_len, :].copy()
            h = jnp.concatenate([mem, xs], axis=1)
            q = jnp.einsum('btd,dhe->bhte', h, Wq)
            k = jnp.einsum('btd,dhe->bhte', h, Wk)
            v = jnp.einsum('btd,dhe->bhte', h, Wv)
            scores = jnp.einsum('bhqe,bhke->bhqk', q, k) * scale
            scores = jnp.where(mask[None, None], scores, -1000000000.0)
            p = _softmax(scores, axis=-1)
            o = jnp.einsum('bhqk,bhke->bhqe', p, v)
            o = jnp.einsum('bhte,hed->btd', o, Wo)
            mem = o[:, :M, :].copy()
            outs.append(o[:, M:, :])
        return jnp.concatenate(outs, axis=1)

    def _B_ref(x, w_gate, w_up, w_down):
        g = jnp.einsum('bsd,df->bsf', x, w_gate)
        u = jnp.einsum('bsd,df->bsf', x, w_up)
        h = _gelu(g) * u
        return jnp.einsum('bsf,fd->bsd', h, w_down)
    x = A_x
    g = _sigmoid((x * gate_w).sum(-1, keepdims=True))
    a = _A_ref(x, A_mem0, A_Wq, A_Wk, A_Wv, A_Wo, A_seg_len)
    b = _B_ref(x, B_w_gate, B_w_up, B_w_down)
    return g * a + (1 - g) * b
```

```python
import jax
import jax.numpy as jnp
import jax.experimental.pallas as pl
import jax.experimental.pallas.tpu as pltpu

S, DM, H, DH, MEM, SEG, DF = 2048, 640, 32, 128, 8, 32, 1728
NSEG = S // SEG
RIDE = SEG - MEM
LEFT = MEM
NL = NSEG * LEFT
BF = jnp.bfloat16
F32 = jnp.float32
U32 = jnp.uint32
NEG = -1000000000.0
NT_FULL = DF // 128
NGU = 2 * NT_FULL + 1
DFP = (NT_FULL + 1) * 128
KT = DM // 128
NCH = 3 * KT
CR = 128 * H
NPR = H // 2
UN = 4

D1, D2, D3 = 1, 2, 1
GSTART, GPER, GLAG = NPR, 4, 1
KB = 7
TPI = 4
LAG = 8
R0 = 3
DBL = (6, 10, 13)

SEM_XL, SEM_X, SEM_GU, SEM_WD, SEM_WO = 0, 1, 2, 3, 4
SEM_W = 5
SEM_OUT = SEM_W + NCH
NSEM = SEM_OUT + 1


def _bf(x):
    return pltpu.bitcast(x, BF)


def _kernel(x_hbm, mem0_ref, wq_hbm, wk_hbm, wv_hbm, wo_hbm, wgt_hbm, wut_hbm, wd_hbm, gw_ref,
            out_hbm,
            x_v, xl_v, xlk_v, wraw_v, gut_s,
            wqkv_v, wo_v, wgu_v, wd_v, left_qkv, left_o, outf_v, outb_v, mem_v, sems):
    scale = DH ** (-0.5)
    w_hbm = (wq_hbm, wk_hbm, wv_hbm)

    def w_copy(k):
        m, c = divmod(k, KT)
        return pltpu.make_async_copy(w_hbm[m].at[c * CR:(c + 1) * CR, :],
                                     wraw_v.at[k * CR:(k + 1) * CR, :], sems.at[SEM_W + k])

    def w_wait(k):
        r = pl.multiple_of(k * CR, CR)
        pltpu.make_async_copy(wraw_v.at[pl.ds(r, CR), :], wraw_v.at[pl.ds(r, CR), :], sems.at[SEM_W + k]).wait()

    xl_copy = pltpu.make_async_copy(x_hbm.at[:, RIDE:SEG, :], xl_v, sems.at[SEM_XL])
    x_copy = pltpu.make_async_copy(x_hbm, x_v, sems.at[SEM_X])
    wd_copy = pltpu.make_async_copy(wd_hbm.bitcast(U32), wd_v.at[0:DF // 2, :], sems.at[SEM_WD])
    wo_copy = pltpu.make_async_copy(wo_hbm.bitcast(U32), wo_v, sems.at[SEM_WO])
    gu_copies = []
    for t in range(NT_FULL):
        for i, src in enumerate((wgt_hbm, wut_hbm)):
            gu_copies.append(pltpu.make_async_copy(src.at[t * 128:(t + 1) * 128, :], gut_s.at[2 * t + i], sems.at[SEM_GU]))
    for i, src in enumerate((wgt_hbm, wut_hbm)):
        gu_copies.append(pltpu.make_async_copy(src.at[NT_FULL * 128:DF, :],
                                               gut_s.at[NGU - 1, i * 64:(i + 1) * 64, :], sems.at[SEM_GU]))

    xl_copy.start()
    for k in range(NCH):
        w_copy(k).start()
        if k == KB + 1:
            for cp in gu_copies:
                cp.start()
    for cp in (wd_copy, x_copy, wo_copy):
        cp.start()

    w32 = wraw_v.bitcast(U32)

    def split(k):
        if isinstance(k, int):
            return divmod(k, KT)
        m = k // KT
        return m, k - m * KT

    def relayout(k, j):
        m, c = split(k)
        blk = w32.at[pl.ds(pl.multiple_of(k * (CR // 2), CR // 2), CR // 2)]
        r0 = pl.multiple_of(c * 64, 64)
        for i in range(8):
            a = blk[pl.ds(i * 256 + j, 8, stride=32), :]
            b = blk[pl.ds(i * 256 + 16 + j, 8, stride=32), :]
            lo = (a & U32(0xFFFF)) | (b << 16)
            hi = (a >> 16) | (b & U32(0xFFFF0000))
            wqkv_v[m, pl.ds(r0 + i * 8, 8), (2 * j) * DH:(2 * j + 1) * DH] = lo
            wqkv_v[m, pl.ds(r0 + i * 8, 8), (2 * j + 1) * DH:(2 * j + 2) * DH] = hi

    def bulk(k, j):
        m, c = split(k)
        xk = _bf(xlk_v[c])
        r0 = pl.multiple_of(c * 64, 64)
        for h in (2 * j, 2 * j + 1):
            cs = slice(h * DH, (h + 1) * DH)
            r = jnp.dot(xk, _bf(wqkv_v[m, pl.ds(r0, 64), cs]), preferred_element_type=F32)
            r = r.reshape(NSEG, LEFT, DH)
            if isinstance(k, int):
                if c > 0:
                    r = r + left_qkv[m, :, :, cs]
            else:
                r = r + jnp.where(c > 0, left_qkv[m, :, :, cs], 0.0)
            left_qkv[m, :, :, cs] = r

    def prep_gu(t):
        wgu_v[t] = pltpu.bitcast(gut_s[t].T, U32)

    wd_v[DF // 2:DFP // 2, :] = jnp.zeros((DFP // 2 - DF // 2, DM), U32)
    mem_v[...] = mem0_ref[0].astype(F32)
    xl_copy.wait()
    xl = xl_v[...].astype(F32).reshape(NL, DM).astype(BF)
    for c in range(KT):
        xlk_v[c] = pltpu.bitcast(xl[:, c * 128:(c + 1) * 128], U32)
    w_wait(0)
    for i in range(NPR):
        relayout(0, i)
        if i < NPR - LAG:
            bulk(0, i)

    def chunk_body(k, with_gu):
        w_wait(k + 1)
        nr = 0
        for i in range(NPR):
            if i >= R0:
                for _ in range(2 if i in DBL else 1):
                    if nr < NPR:
                        relayout(k + 1, nr)
                        nr += 1
            if with_gu and i % (NPR // TPI) == 0:
                prep_gu(jnp.minimum((k - KB) * TPI + i // (NPR // TPI), NGU - 1))
            if i < LAG:
                bulk(k, NPR - LAG + i)
            else:
                bulk(k + 1, i - LAG)
        assert nr == NPR

    def body_a(k, c):
        chunk_body(k, False)
        return c

    def body_b(k, c):
        chunk_body(k, True)
        return c

    jax.lax.fori_loop(0, KB, body_a, 0)
    pltpu.make_async_copy(gut_s, gut_s, sems.at[SEM_GU]).wait()
    jax.lax.fori_loop(KB, NCH - 1, body_b, 0)
    for i in range(NPR - LAG, NPR):
        bulk(NCH - 1, i)
    x_copy.wait()
    wd_copy.wait()
    wo_copy.wait()

    L = SEG + MEM
    qi = jax.lax.broadcasted_iota(jnp.int32, (2 * L, 128), 0)
    ki = jax.lax.broadcasted_iota(jnp.int32, (2 * L, 128), 1)
    q2 = qi >= L
    k2 = ki >= L
    ql = jnp.where(q2, qi - L, qi)
    kl = jnp.where(k2, ki - L, ki)
    q_mem = (ql >= RIDE) & (ql < SEG)
    k_mem = (kl >= RIDE) & (kl < SEG)
    mask = (ki < 2 * L) & (q2 == k2) & (q_mem | k_mem | (kl <= ql))

    gw = gw_ref[...].astype(F32)

    def step(s, u):
        xs = x_v[s]
        xf = xs.astype(F32)
        lhs = jnp.concatenate([xf[:RIDE], mem_v[...]], axis=0).astype(BF)
        zpad = jnp.zeros((128 - 2 * L, DH), F32)
        st = {}
        gate = jax.nn.sigmoid(jnp.sum(xf * gw, axis=-1, keepdims=True))
        gate = jnp.broadcast_to(gate, (SEG, 128))
        one8 = jnp.ones((8, 128), F32)
        gfac = jnp.concatenate([gate[:RIDE], one8, gate[RIDE:]] * 2, axis=0)
        ngate = 1.0 - gate

        def qkv_stage(j):
            parts = []
            for h in (2 * j, 2 * j + 1):
                ch = slice(h * DH, (h + 1) * DH)
                w = jnp.concatenate([wqkv_v[m, :, ch] for m in range(3)], axis=1)
                qkv = jnp.dot(lhs, _bf(w), preferred_element_type=F32)
                parts.append([(qkv[:, m * DH:(m + 1) * DH], left_qkv[m, s, :, ch]) for m in range(3)])
            q = jnp.concatenate([*parts[0][0], *parts[1][0]], axis=0).astype(BF)
            k = jnp.concatenate([*parts[0][1], *parts[1][1], zpad], axis=0).astype(BF)
            v = jnp.concatenate([*parts[0][2], *parts[1][2], zpad], axis=0).astype(BF)
            st[j] = (q, k, v)

        def score_stage(j):
            q, k, v = st[j]
            sc = jax.lax.dot_general(q, k, (((1,), (1,)), ((), ())), preferred_element_type=F32) * scale
            sc = jnp.where(mask, sc, NEG)
            m = jnp.max(sc, axis=-1, keepdims=True)
            p = jnp.exp(sc - m)
            l = jnp.sum(p, axis=-1, keepdims=True)
            r = pl.reciprocal(l, approx=True)
            r = r * (2.0 - l * r)
            p = p * (r * gfac)
            st[j] = (p.astype(BF), v)

        def pv_stage(j):
            p, v = st[j]
            o = jnp.dot(p, v, preferred_element_type=F32)
            cs = slice(2 * j * DH, (2 * j + 2) * DH)
            o = jnp.concatenate([o[:L], o[L:]], axis=1)
            if u < UN - 1:
                left_o[u, :, cs] = o[SEG:]
                st[j] = o[:SEG].astype(BF)
            else:
                st[j] = jnp.concatenate([o[:SEG]] + [left_o[w, :, cs] for w in range(UN - 1)] + [o[SEG:]],
                                        axis=0).astype(BF)

        def wo_stage(j):
            r = jnp.dot(st.pop(j), _bf(wo_v[j * 128:(j + 1) * 128, :]), preferred_element_type=F32)
            st['acc'] = r if 'acc' not in st else st['acc'] + r

        def gu_stage(t):
            if t < NT_FULL:
                w = jnp.concatenate([wgu_v[2 * t], wgu_v[2 * t + 1]], axis=1)
                gu = jnp.dot(xs, _bf(w), preferred_element_type=F32)
                g_, u_ = gu[:, :128], gu[:, 128:]
            else:
                g_ = jnp.dot(xs, _bf(wgu_v[2 * t]), preferred_element_type=F32)
                u_ = pltpu.roll(g_, 64, 1)
            st[('h', t)] = (jax.nn.gelu(g_, approximate=True) * (u_ * ngate)).astype(BF)

        def down_stage(t):
            r = jnp.dot(st.pop(('h', t)), _bf(wd_v[t * 64:(t + 1) * 64, :]), preferred_element_type=F32)
            st['b'] = r if 'b' not in st else st['b'] + r

        depth = D1 + D2 + D3
        ngut = NT_FULL + 1
        nslot = NPR + depth + GLAG + 2
        gu_sched = {i: [] for i in range(-GLAG, nslot)}
        for t in range(ngut):
            gu_sched[GSTART + t // GPER].append(t)
        for i in range(nslot):
            if i < NPR:
                qkv_stage(i)
            for t in gu_sched[i]:
                gu_stage(t)
            if 0 <= i - D1 < NPR:
                score_stage(i - D1)
            if 0 <= i - D1 - D2 < NPR:
                pv_stage(i - D1 - D2)
            if 0 <= i - depth < NPR:
                wo_stage(i - depth)
            for t in gu_sched[i - GLAG]:
                down_stage(t)

        acc = st['acc']
        b = st['b']
        mem_v[...] = acc[RIDE:SEG].astype(BF).astype(F32)
        outb_v[s, 0:16, :] = (acc[:16] + b[:16]).astype(BF)
        hi = jnp.concatenate([acc[16:RIDE] + b[16:RIDE], b[RIDE:]], axis=0)
        if u < UN - 1:
            outf_v[u] = hi
        else:
            for w in range(UN):
                hw = hi if w == UN - 1 else outf_v[w]
                al = acc[SEG + w * LEFT:SEG + (w + 1) * LEFT]
                outb_v[s - (UN - 1) + w, 16:SEG, :] = jnp.concatenate([hw[:8], hw[8:] + al], axis=0).astype(BF)

    def group(i, carry):
        for u in range(UN):
            step(i * UN + u, u)
        sl = pl.ds(pl.multiple_of(i * UN, UN), UN)
        pltpu.make_async_copy(outb_v.at[sl], out_hbm.at[sl], sems.at[SEM_OUT]).start()
        return carry

    jax.lax.fori_loop(0, NSEG // UN, group, 0)
    pltpu.make_async_copy(outb_v, out_hbm, sems.at[SEM_OUT]).wait()


@jax.jit
def pallas_gated_mix__memory_aug_recurrent_mem_tr__glu_gated_geglu__prompt_kernel(
    A_x, A_mem0, A_Wq, A_Wk, A_Wv, A_Wo, A_seg_len, B_x, B_w_gate, B_w_up, B_w_down, gate_w,
):
    x = A_x.reshape(NSEG, SEG, DM)
    wq = A_Wq.reshape(DM * H, DH)
    wk = A_Wk.reshape(DM * H, DH)
    wv = A_Wv.reshape(DM * H, DH)
    wo = A_Wo.reshape(H * DH, DM)
    gw = gate_w.reshape(1, DM)
    anyspec = pl.BlockSpec(memory_space=pl.ANY)
    vmem = pl.BlockSpec(memory_space=pltpu.VMEM)
    out = pl.pallas_call(
        _kernel,
        out_shape=jax.ShapeDtypeStruct((NSEG, SEG, DM), BF),
        in_specs=[anyspec, vmem, anyspec, anyspec, anyspec, anyspec, anyspec, anyspec, anyspec, vmem],
        out_specs=anyspec,
        scratch_shapes=[
            pltpu.VMEM((NSEG, SEG, DM), BF),
            pltpu.VMEM((NSEG, LEFT, DM), BF),
            pltpu.VMEM((KT, NL // 2, 128), U32),
            pltpu.VMEM((3 * DM * H, DH), BF),
            pltpu.VMEM((NGU, 128, DM), BF),
            pltpu.VMEM((3, DM // 2, H * DH), U32),
            pltpu.VMEM((H * DH // 2, DM), U32),
            pltpu.VMEM((NGU, DM // 2, 128), U32),
            pltpu.VMEM((DFP // 2, DM), U32),
            pltpu.VMEM((3, NSEG, LEFT, H * DH), F32),
            pltpu.VMEM((UN - 1, LEFT, H * DH), F32),
            pltpu.VMEM((UN - 1, 16, DM), F32),
            pltpu.VMEM((NSEG, SEG, DM), BF),
            pltpu.VMEM((MEM, DM), F32),
            pltpu.SemaphoreType.DMA((NSEM,)),
        ],
        compiler_params=pltpu.CompilerParams(vmem_limit_bytes=124 * 1024 * 1024),
    )(x, A_mem0, wq, wk, wv, wo, B_w_gate.T, B_w_up.T, B_w_down, gw)
    return out.reshape(1, S, DM)
```

```python
import jax
import jax.numpy as jnp
import jax.experimental.pallas as pl
import jax.experimental.pallas.tpu as pltpu

S, DM, H, DH, MEM, SEG, DF = 2048, 640, 32, 128, 8, 32, 1728
NSEG = S // SEG
RIDE = SEG - MEM
LEFT = MEM
NL = NSEG * LEFT
BF = jnp.bfloat16
F32 = jnp.float32
U32 = jnp.uint32
NEG = -1000000000.0
NT_FULL = DF // 128
NGU = 2 * NT_FULL + 1
DFP = (NT_FULL + 1) * 128
KT = DM // 128
NCH = 3 * KT
CR = 128 * H
NPR = H // 2
UN = 4

D1, D2, D3 = 1, 2, 1
GSTART, GPER, GLAG = NPR, 4, 1
KA = 2
NB = (NCH - 1 - KA) // 2
TPI = 5
NGP = NB * TPI
LAG = 6
R0 = 3
DBL = (6, 10, 13)

SEM_XL0, SEM_XL, SEM_X, SEM_WD, SEM_WO, SEM_M0, SEM_GW = range(7)
SEM_GU = 7
SEM_W = SEM_GU + NB
SEM_OUT = SEM_W + NCH
NSEM = SEM_OUT + 1


def _bf(x):
    return pltpu.bitcast(x, BF)


def _kernel(x_hbm, mem0_hbm, wq_hbm, wk_hbm, wv_hbm, wo_hbm, wgt_hbm, wut_hbm, wd_hbm, gw_hbm,
            out_hbm,
            x_v, xl_v, xlk_v, mem0_v, gw_v, wraw_v, gut_s,
            wqkv_v, wo_v, wgu_v, wd_v, left_qkv, left_o, outf_v, outb_v, mem_v, sems):
    scale = DH ** (-0.5)
    w_hbm = (wq_hbm, wk_hbm, wv_hbm)

    def w_copy(k):
        c, m = divmod(k, 3)
        return pltpu.make_async_copy(w_hbm[m].at[c * CR:(c + 1) * CR, :],
                                     wraw_v.at[k * CR:(k + 1) * CR, :], sems.at[SEM_W + k])

    def w_wait(k):
        r = pl.multiple_of(k * CR, CR)
        pltpu.make_async_copy(wraw_v.at[pl.ds(r, CR), :], wraw_v.at[pl.ds(r, CR), :], sems.at[SEM_W + k]).wait()

    xl_copies = [pltpu.make_async_copy(x_hbm.at[:, RIDE:SEG, c * 128:(c + 1) * 128], xl_v.at[c],
                                       sems.at[SEM_XL if c else SEM_XL0]) for c in range(KT)]
    m0_copy = pltpu.make_async_copy(mem0_hbm, mem0_v, sems.at[SEM_M0])
    gw_copy = pltpu.make_async_copy(gw_hbm, gw_v, sems.at[SEM_GW])
    x_copy = pltpu.make_async_copy(x_hbm, x_v, sems.at[SEM_X])
    wd_copy = pltpu.make_async_copy(wd_hbm.bitcast(U32), wd_v.at[0:DF // 2, :], sems.at[SEM_WD])
    wo_copy = pltpu.make_async_copy(wo_hbm.bitcast(U32), wo_v, sems.at[SEM_WO])
    gu_copies = [[] for _ in range(NB)]
    for slot in range(NGP):
        sem = sems.at[SEM_GU + slot // TPI]
        if slot == NGU - 1:
            for i, src in enumerate((wgt_hbm, wut_hbm)):
                gu_copies[slot // TPI].append(pltpu.make_async_copy(
                    src.at[NT_FULL * 128:DF, :], gut_s.at[slot, i * 64:(i + 1) * 64, :], sem))
        else:
            t, i = divmod(slot % (NGU - 1), 2)
            gu_copies[slot // TPI].append(pltpu.make_async_copy(
                (wgt_hbm, wut_hbm)[i].at[t * 128:(t + 1) * 128, :], gut_s.at[slot], sem))

    xl_copies[0].start()
    for k in range(NCH):
        w_copy(k).start()
        if k == KA:
            for cp in xl_copies[1:]:
                cp.start()
        if k > KA and (k - KA) % 2 == 0:
            for cp in gu_copies[(k - KA) // 2 - 1]:
                cp.start()
    for cp in (m0_copy, gw_copy, wd_copy, x_copy, wo_copy):
        cp.start()

    w32 = wraw_v.bitcast(U32)

    def split(k):
        c = k // 3
        return k - c * 3, c

    def relayout(k, j):
        m, c = split(k)
        blk = w32.at[pl.ds(pl.multiple_of(k * (CR // 2), CR // 2), CR // 2)]
        r0 = pl.multiple_of(c * 64, 64)
        for i in range(8):
            a = blk[pl.ds(i * 256 + j, 8, stride=32), :]
            b = blk[pl.ds(i * 256 + 16 + j, 8, stride=32), :]
            lo = (a & U32(0xFFFF)) | (b << 16)
            hi = (a >> 16) | (b & U32(0xFFFF0000))
            wqkv_v[m, pl.ds(r0 + i * 8, 8), (2 * j) * DH:(2 * j + 1) * DH] = lo
            wqkv_v[m, pl.ds(r0 + i * 8, 8), (2 * j + 1) * DH:(2 * j + 2) * DH] = hi

    def bulk(k, j):
        m, c = split(k)
        xk = _bf(xlk_v[c])
        r0 = pl.multiple_of(c * 64, 64)
        for h in (2 * j, 2 * j + 1):
            cs = slice(h * DH, (h + 1) * DH)
            r = jnp.dot(xk, _bf(wqkv_v[m, pl.ds(r0, 64), cs]), preferred_element_type=F32)
            r = r.reshape(NSEG, LEFT, DH)
            if isinstance(k, int):
                if c > 0:
                    r = r + left_qkv[m, :, :, cs]
            else:
                r = r + jnp.where(c > 0, left_qkv[m, :, :, cs], 0.0)
            left_qkv[m, :, :, cs] = r

    def prep_gu(t):
        wgu_v[t] = pltpu.bitcast(gut_s[t].T, U32)

    wd_v[DF // 2:DFP // 2, :] = jnp.zeros((DFP // 2 - DF // 2, DM), U32)
    def pack_xl(c):
        xlk_v[c] = pltpu.bitcast(xl_v[c].reshape(NL, 128), U32)

    xl_copies[0].wait()
    pack_xl(0)
    w_wait(0)
    for i in range(NPR):
        relayout(0, i)
        if i < NPR - LAG:
            bulk(0, i)

    def chunk_body(k, n, gu0):
        nr = 0
        for i in range(n * NPR):
            if i >= R0:
                for _ in range(2 if i in DBL else 1):
                    relayout(k + 1 + nr // NPR, nr % NPR)
                    nr += 1
            if gu0 is not None and i % 6 == 0 and i // 6 < TPI:
                prep_gu(gu0 + i // 6)
            q = i + NPR - LAG
            bulk(k + q // NPR, q % NPR)
        assert nr == n * NPR

    def body_a(k, c):
        w_wait(k + 1)
        chunk_body(k, 1, None)
        return c

    def body_b(kk, c):
        k = KA + 2 * kk
        w_wait(k + 1)
        w_wait(k + 2)
        g0 = pl.multiple_of(kk * TPI, TPI)
        pltpu.make_async_copy(gut_s.at[pl.ds(g0, TPI)], gut_s.at[pl.ds(g0, TPI)], sems.at[SEM_GU + kk]).wait()
        chunk_body(k, 2, g0)
        return c

    jax.lax.fori_loop(0, KA, body_a, 0)
    pltpu.make_async_copy(xl_v.at[1:KT], xl_v.at[1:KT], sems.at[SEM_XL]).wait()
    for c in range(1, KT):
        pack_xl(c)
    jax.lax.fori_loop(0, NB, body_b, 0)
    for i in range(NPR - LAG, NPR):
        bulk(NCH - 1, i)
    for cp in (m0_copy, gw_copy, wd_copy, x_copy, wo_copy):
        cp.wait()
    mem_v[...] = mem0_v[0].astype(F32)

    L = SEG + MEM
    qi = jax.lax.broadcasted_iota(jnp.int32, (2 * L, 128), 0)
    ki = jax.lax.broadcasted_iota(jnp.int32, (2 * L, 128), 1)
    q2 = qi >= L
    k2 = ki >= L
    ql = jnp.where(q2, qi - L, qi)
    kl = jnp.where(k2, ki - L, ki)
    q_mem = (ql >= RIDE) & (ql < SEG)
    k_mem = (kl >= RIDE) & (kl < SEG)
    own = (ki < 2 * L) & (q2 == k2)
    mask = own & (q_mem | k_mem | (kl <= ql))
    fill = jnp.where(own, NEG, -jnp.inf).astype(F32)
    half = jax.lax.broadcasted_iota(jnp.int32, (SEG, 128), 1) < 64

    gw = gw_v[...].astype(F32).reshape(1, DM)

    def step(s, u):
        xs = x_v[s]
        xf = xs.astype(F32)
        lhs = jnp.concatenate([xf[:RIDE], mem_v[...]], axis=0).astype(BF)
        zpad = jnp.zeros((128 - 2 * L, DH), F32)
        st = {}
        gate = jax.nn.sigmoid(jnp.sum(xf * gw, axis=-1, keepdims=True))
        gate = jnp.broadcast_to(gate, (SEG, 128))
        one8 = jnp.ones((8, 128), F32)
        gfac = jnp.concatenate([gate[:RIDE], one8, gate[RIDE:]] * 2, axis=0)
        ngate = 1.0 - gate

        def qkv_stage(j):
            parts = []
            for h in (2 * j, 2 * j + 1):
                ch = slice(h * DH, (h + 1) * DH)
                w = jnp.concatenate([wqkv_v[m, :, ch] for m in range(3)], axis=1)
                qkv = jnp.dot(lhs, _bf(w), preferred_element_type=F32)
                parts.append([(qkv[:, m * DH:(m + 1) * DH], left_qkv[m, s, :, ch]) for m in range(3)])
            q = jnp.concatenate([*parts[0][0], *parts[1][0]], axis=0).astype(BF)
            k = jnp.concatenate([*parts[0][1], *parts[1][1], zpad], axis=0).astype(BF)
            v = jnp.concatenate([*parts[0][2], *parts[1][2], zpad], axis=0).astype(BF)
            st[j] = (q, k, v)

        def score_stage(j):
            q, k, v = st[j]
            sc = jax.lax.dot_general(q, k, (((1,), (1,)), ((), ())), preferred_element_type=F32) * scale
            sc = jnp.where(mask, sc, fill)
            m = jnp.max(sc, axis=-1, keepdims=True)
            p = jnp.exp(sc - m)
            l = jnp.sum(p, axis=-1, keepdims=True)
            r = pl.reciprocal(l, approx=True)
            r = r * (2.0 - l * r)
            p = p * (r * gfac)
            st[j] = (p.astype(BF), v)

        def pv_stage(j):
            p, v = st[j]
            o = jnp.dot(p, v, preferred_element_type=F32)
            cs = slice(2 * j * DH, (2 * j + 2) * DH)
            o = jnp.concatenate([o[:L], o[L:]], axis=1)
            if u < UN - 1:
                left_o[u, :, cs] = o[SEG:]
                st[j] = o[:SEG].astype(BF)
            else:
                st[j] = jnp.concatenate([o[:SEG]] + [left_o[w, :, cs] for w in range(UN - 1)] + [o[SEG:]],
                                        axis=0).astype(BF)

        def wo_stage(j):
            r = jnp.dot(st.pop(j), _bf(wo_v[j * 128:(j + 1) * 128, :]), preferred_element_type=F32)
            st['acc'] = r if 'acc' not in st else st['acc'] + r

        def gu_stage(t):
            if t < NT_FULL:
                w = jnp.concatenate([wgu_v[2 * t], wgu_v[2 * t + 1]], axis=1)
                gu = jnp.dot(xs, _bf(w), preferred_element_type=F32)
                g_, u_ = gu[:, :128], gu[:, 128:]
            else:
                g_ = jnp.dot(xs, _bf(wgu_v[2 * t]), preferred_element_type=F32)
                u_ = pltpu.roll(g_, 64, 1)
            hh = jax.nn.gelu(g_, approximate=True) * (u_ * ngate)
            if t == NT_FULL:
                hh = jnp.where(half, hh, 0.0)
            st[('h', t)] = hh.astype(BF)

        def down_stage(t):
            r = jnp.dot(st.pop(('h', t)), _bf(wd_v[t * 64:(t + 1) * 64, :]), preferred_element_type=F32)
            st['b'] = r if 'b' not in st else st['b'] + r

        depth = D1 + D2 + D3
        ngut = NT_FULL + 1
        nslot = NPR + depth + GLAG + 2
        gu_sched = {i: [] for i in range(-GLAG, nslot)}
        for t in range(ngut):
            gu_sched[GSTART + t // GPER].append(t)
        for i in range(nslot):
            if i < NPR:
                qkv_stage(i)
            for t in gu_sched[i]:
                gu_stage(t)
            if 0 <= i - D1 < NPR:
                score_stage(i - D1)
            if 0 <= i - D1 - D2 < NPR:
                pv_stage(i - D1 - D2)
            if 0 <= i - depth < NPR:
                wo_stage(i - depth)
            for t in gu_sched[i - GLAG]:
                down_stage(t)

        acc = st['acc']
        b = st['b']
        mem_v[...] = acc[RIDE:SEG].astype(BF).astype(F32)
        outb_v[s, 0:16, :] = (acc[:16] + b[:16]).astype(BF)
        hi = jnp.concatenate([acc[16:RIDE] + b[16:RIDE], b[RIDE:]], axis=0)
        if u < UN - 1:
            outf_v[u] = hi
        else:
            for w in range(UN):
                hw = hi if w == UN - 1 else outf_v[w]
                al = acc[SEG + w * LEFT:SEG + (w + 1) * LEFT]
                outb_v[s - (UN - 1) + w, 16:SEG, :] = jnp.concatenate([hw[:8], hw[8:] + al], axis=0).astype(BF)

    def group(i, carry):
        for u in range(UN):
            step(i * UN + u, u)
        sl = pl.ds(pl.multiple_of(i * UN, UN), UN)
        pltpu.make_async_copy(outb_v.at[sl], out_hbm.at[sl], sems.at[SEM_OUT]).start()
        return carry

    jax.lax.fori_loop(0, NSEG // UN, group, 0)
    pltpu.make_async_copy(outb_v, out_hbm, sems.at[SEM_OUT]).wait()


@jax.jit
def pallas_gated_mix__memory_aug_recurrent_mem_tr__glu_gated_geglu__prompt_kernel(
    A_x, A_mem0, A_Wq, A_Wk, A_Wv, A_Wo, A_seg_len, B_x, B_w_gate, B_w_up, B_w_down, gate_w,
):
    x = A_x.reshape(NSEG, SEG, DM)
    wq = A_Wq.reshape(DM * H, DH)
    wk = A_Wk.reshape(DM * H, DH)
    wv = A_Wv.reshape(DM * H, DH)
    wo = A_Wo.reshape(H * DH, DM)
    anyspec = pl.BlockSpec(memory_space=pl.ANY)
    out = pl.pallas_call(
        _kernel,
        out_shape=jax.ShapeDtypeStruct((NSEG, SEG, DM), BF),
        in_specs=[anyspec] * 10,
        out_specs=anyspec,
        scratch_shapes=[
            pltpu.VMEM((NSEG, SEG, DM), BF),
            pltpu.VMEM((KT, NSEG, LEFT, 128), BF),
            pltpu.VMEM((KT, NL // 2, 128), U32),
            pltpu.VMEM((1, MEM, DM), BF),
            pltpu.VMEM((DM,), BF),
            pltpu.VMEM((3 * DM * H, DH), BF),
            pltpu.VMEM((NGP, 128, DM), BF),
            pltpu.VMEM((3, DM // 2, H * DH), U32),
            pltpu.VMEM((H * DH // 2, DM), U32),
            pltpu.VMEM((NGP, DM // 2, 128), U32),
            pltpu.VMEM((DFP // 2, DM), U32),
            pltpu.VMEM((3, NSEG, LEFT, H * DH), F32),
            pltpu.VMEM((UN - 1, LEFT, H * DH), F32),
            pltpu.VMEM((UN - 1, 16, DM), F32),
            pltpu.VMEM((NSEG, SEG, DM), BF),
            pltpu.VMEM((MEM, DM), F32),
            pltpu.SemaphoreType.DMA((NSEM,)),
        ],
        compiler_params=pltpu.CompilerParams(vmem_limit_bytes=100 * 1024 * 1024),
    )(x, A_mem0, wq, wk, wv, wo, B_w_gate.T, B_w_up.T, B_w_down, gate_w)
    return out.reshape(1, S, DM)
```
